```python
import os as _os
_os.environ.setdefault("JAX_PLATFORMS", "cpu")
import jax
import jax.numpy as jnp

def _softmax(x, axis=-1):
    return jax.nn.softmax(x, axis=axis)
def _gelu(x):
    return jax.nn.gelu(x, approximate=True)
def _silu(x):
    return jax.nn.silu(x)
def _sigmoid(x):
    return jax.nn.sigmoid(x)
def _layernorm(x, axis=-1, eps=1e-5):
    m = jnp.mean(x, axis=axis, keepdims=True)
    v = jnp.var(x, axis=axis, keepdims=True)
    return (x - m) / jnp.sqrt(v + eps)
def _scatter_add(tgt, idx, src, axis=0):
    return tgt.at[idx].add(src)
def _segment_sum(src, seg, n):
    return jax.ops.segment_sum(src, seg, n)
class _Rng:
    def __init__(self, key):
        self._k = key
    def _next(self):
        self._k, sub = jax.random.split(self._k)
        return sub
    def normal(self, shape):
        return jax.random.normal(self._next(), shape, dtype=jnp.bfloat16)
    def randint(self, lo, hi, shape):
        return jax.random.randint(self._next(), shape, lo, hi, dtype=jnp.int32)
    def uniform(self, shape, lo=0.0, hi=1.0):
        return jax.random.uniform(self._next(), shape, jnp.bfloat16, lo, hi)
    def permutation(self, n):
        return jax.random.permutation(self._next(), n)


kernel_name = 'sequential_preLN__ssm_conv_h3__mixer_s_mlp__prompt'

def setup_inputs():
    _rng = _Rng(jax.random.key(int.from_bytes(__import__("os").urandom(4), "little")))
    _w = (lambda a: (lambda t: t.astype(jnp.bfloat16) if jnp.issubdtype(t.dtype, jnp.floating) else t)(jnp.asarray(a)))
    def _A_setup():
        B, S, D = 1, 2048, 640
        ks = 4
        return {
            "q": _w((lambda *s: _rng.normal(s) * 0.05)(B, S, D)),
            "k": _w((lambda *s: _rng.normal(s) * 0.05)(B, S, D)),
            "v": _w((lambda *s: _rng.normal(s) * 0.05)(B, S, D)),
            "shift_k": _w((lambda *s: _rng.normal(s) * 0.05)(D, ks) * 0.5),
            "ssm_k": _w((lambda *s: _rng.normal(s) * 0.05)(D, S) * (1.0 / S ** 0.5)),
            "ssm_D": _w((lambda *s: _rng.normal(s) * 0.05)(D)),
        }
    _A_in = _A_setup()

    def _B_setup():
        B, S, D, F = 1, 2048, 640, 1728
        return {
            "x":  _w((lambda *s: _rng.normal(s) * 0.05)(B, S, D)),
            "w1": _w((lambda *s: _rng.normal(s) * 0.8)(D, D) * (D ** -0.5)),
            "w2": _w((lambda *s: _rng.normal(s) * 0.8)(D, D) * (D ** -0.5)),
            "w3": _w((lambda *s: _rng.normal(s) * 0.8)(D, F) * (D ** -0.5)),
            "w4": _w((lambda *s: _rng.normal(s) * 0.8)(F, D) * (F ** -0.5)),
        }
    _B_in = _B_setup()

    return {
        "A_q": _A_in["q"],
        "A_k": _A_in["k"],
        "A_v": _A_in["v"],
        "A_shift_k": _A_in["shift_k"],
        "A_ssm_k": _A_in["ssm_k"],
        "A_ssm_D": _A_in["ssm_D"],
        "B_x": _B_in["x"],
        "B_w1": _B_in["w1"],
        "B_w2": _B_in["w2"],
        "B_w3": _B_in["w3"],
        "B_w4": _B_in["w4"],
    }

def reference(A_q, A_k, A_v, A_shift_k, A_ssm_k, A_ssm_D, B_x, B_w1, B_w2, B_w3, B_w4):
    def _A_ref(q, k, v, shift_k, ssm_k, ssm_D):
        B, S, D = q.shape
        ks = shift_k.shape[-1]
        k_pad = jnp.pad(k, ((0, 0), (ks - 1, 0), (0, 0)))
        k_shift = jnp.zeros_like(k)
        for t in range(ks):
            k_shift = k_shift + k_pad[:, t:t + S, :] * shift_k[:, ks - 1 - t][None, None, :]
        kv = k_shift * v
        L = 2 * S
        kv_pad = jnp.pad(kv, ((0, 0), (0, S), (0, 0)))
        kf_pad = jnp.pad(ssm_k, ((0, 0), (0, S)))
        kv_f = (lambda x, axes=(-2,-1): jnp.fft.rfft2(x.astype(jnp.float32), axes=axes))(kv_pad[:, None, :, :], axes=(1, 2))
        kf_f = (lambda x, axes=(-2,-1): jnp.fft.rfft2(x.astype(jnp.float32), axes=axes))(kf_pad[:, None, :], axes=(1, 2))
        kf_f = (lambda x, *d: x.transpose(*d))(kf_f, 1, 2, 0)
        y_f = kv_f * kf_f[None, :, :, :]
        y = (lambda x, s, axes=(-2,-1): jnp.fft.irfft2(x, s=s, axes=axes).astype(jnp.bfloat16))(y_f, (1, L), axes=(1, 2))[:, 0, :S, :]
        y = y + kv * ssm_D[None, None, :]
        return q * y

    def _B_ref(x, w1, w2, w3, w4):
        B, S, D = x.shape
        h = _gelu(_layernorm(x, axis=-1) @ w1)
        c = D // 4
        g0 = jnp.pad(h[:, :, 0*c:1*c], ((0, 0), (1, 0), (0, 0)))[:, :S, :]
        g1 = jnp.pad(h[:, :, 1*c:2*c], ((0, 0), (0, 1), (0, 0)))[:, 1:, :]
        g2 = jnp.pad(h[:, :, 2*c:3*c], ((0, 0), (2, 0), (0, 0)))[:, :S, :]
        g3 = jnp.pad(h[:, :, 3*c:   ], ((0, 0), (0, 2), (0, 0)))[:, 2:, :]
        hs = jnp.concatenate([g0, g1, g2, g3], axis=-1) @ w2
        x1 = x + hs
        h2 = _gelu(_layernorm(x1, axis=-1) @ w3) @ w4
        return x1 + h2

    x = A_q
    h = x + _A_ref(_layernorm(x, axis=-1), A_k, A_v, A_shift_k, A_ssm_k, A_ssm_D)
    h2 = h + _B_ref(_layernorm(h, axis=-1), B_w1, B_w2, B_w3, B_w4)
    return h2
```

```python
import functools
import numpy as np
import jax
import jax.numpy as jnp
import jax.experimental.pallas as pl
import jax.experimental.pallas.tpu as pltpu

S, D, F, KS = 2048, 640, 1728, 4
C = 128
NC = S // C
EPS = 1e-5
NL = D // 128
FP = 1792
NF = FP // 128


def _dft_mats():
    perm = np.concatenate([np.arange(0, C, 2), np.arange(1, C, 2)])
    t = np.arange(C)
    ang = np.outer(2 * perm + 1, t) % (4 * C)
    ang = np.pi * ang / (2 * C)
    fwd = np.concatenate([np.cos(ang), -np.sin(ang)], 0)
    inv = fwd.T / C
    return fwd.astype(np.float32), inv.astype(np.float32)


_FWD, _INV = _dft_mats()
f32, bf16, u32 = jnp.float32, jnp.bfloat16, jnp.uint32


def _gelu(x):
    c0 = float(np.sqrt(2.0 / np.pi))
    c1 = float(np.sqrt(2.0 / np.pi) * 0.044715)
    hx = 0.5 * x
    return hx * jnp.tanh(x * (c0 + c1 * (x * x))) + hx


def _center(x):
    m = jnp.sum(x, axis=-1, keepdims=True) * (1.0 / D)
    d = x - m
    v = jnp.sum(d * d, axis=-1, keepdims=True) * (1.0 / D)
    return d, v

H_W1, H_W2, H_W3, H_W4 = 0, D, 2 * D, 2 * D + FP
WROWS = 2 * D + 2 * FP
PS = C + 8
SROWS = NC * 6 * PS + 8


def build(T=256, lag=3, lag2=2, nodma=0, small=1, wmode=0, only=0, flat=0):
    NS = S // T
    CPS = T // C
    FR = 8

    def body(q_hbm, k_hbm, v_hbm, sk_hbm, w1_hbm, w2_hbm, w3_hbm, w4_hbm,
             shk_hbm, sd_hbm, f_hbm, fi_hbm, z_hbm,
             out_hbm,
             q_v, k_v, v_v, sk_v, wst, shk_ref, sd_ref, f_ref, fi_ref, z_ref,
             sb, wf, kvf, kf_v, kraw_v, h_v, hn_v, g_v, x1_v, out_v, sems, osems):

        class Multi:
            def __init__(self, cs): self.cs = cs
            def start(self):
                if nodma: return
                for c in self.cs: c.start()
            def wait(self):
                if nodma: return
                for c in self.cs: c.wait()

        def tcopy(src, rows, dst, drows, sem):
            return Multi([pltpu.make_async_copy(src.at[rows, pl.ds(t * 128, 128)], dst.at[t, drows], sem) for t in range(NL)])
        def in_copies(s):
            rows = pl.ds(s * T, T)
            return [
                tcopy(k_hbm, rows, k_v, rows, sems.at[s, 0]),
                tcopy(v_hbm, rows, v_v, rows, sems.at[s, 1]),
                Multi([pltpu.make_async_copy(sk_hbm.at[:, pl.ds((s * CPS + cc) * C, C)], sk_v.at[s * CPS + cc], sems.at[s, 2]) for cc in range(CPS)]),
                tcopy(q_hbm, rows, q_v, rows, sems.at[s, 3]),
            ]
        def wcopy(src, off, n, i):
            return tcopy(src, pl.ds(0, n), wst, pl.ds(off, n), sems.at[NS, i])
        wcp = [wcopy(w1_hbm, H_W1, D, 0), wcopy(w2_hbm, H_W2, D, 1), wcopy(w3_hbm, H_W3, F, 2), wcopy(w4_hbm, H_W4, F, 3)]
        ccp = Multi([pltpu.make_async_copy(a, b, sems.at[NS + 1, 0]) for a, b in
                     ((shk_hbm, shk_ref), (sd_hbm, sd_ref), (f_hbm, f_ref), (fi_hbm.at[:, pl.ds(0, 128)], fi_ref.at[0]),
                      (fi_hbm.at[:, pl.ds(128, 128)], fi_ref.at[1]), (z_hbm, z_ref))])
        def out_copy(s):
            rows = pl.ds(s * T, T)
            return Multi([pltpu.make_async_copy(out_v.at[t, rows], out_hbm.at[rows, pl.ds(t * 128, 128)], osems.at[s]) for t in range(NL)])

        ccp.start()
        ins = [in_copies(s) for s in range(NS)]
        for c in ins[0]: c.start()
        for c in ins[1][:3]: c.start()
        wcp[0].start()
        ins[1][3].start()
        def issue(s):
            if s < NS:
                for c in ins[s][:3]: c.start()
                if 2 <= s <= 4: wcp[s - 1].start()
                ins[s][3].start()

        g_v[:, pl.ds(0, 8), :] = jnp.zeros((NL, 8, 128), f32)
        g_v[:, pl.ds(S + 8, 8), :] = jnp.zeros((NL, 8, 128), f32)
        kf_v[:, pl.ds(0, 8), :] = jnp.zeros((NL, 8, 128), f32)
        wst[:, pl.ds(H_W3 + F, FP - F), :] = jnp.zeros((NL, FP - F, 128), bf16)
        wst[:, pl.ds(H_W4 + F, FP - F), :] = jnp.zeros((NL, FP - F, 128), bf16)
        ccp.wait()
        z = z_ref[0]
        if only:
            allc = [c for s in range(NS) for c in ins[s]] + wcp
            order = [c for c in ins[0]] + ins[1][:3] + [wcp[0], ins[1][3]] + ins[2][:3] + [wcp[1], ins[2][3]] + ins[3][:3] + [wcp[2], ins[3][3]] + ins[4][:3] + [wcp[3], ins[4][3]] + [c for s in range(5, NS) for c in ins[s]]
            for c in order[:only]: c.wait()
            pl.delay(30000)
            for c in order[only:]: c.wait()
            return

        wv = wst.bitcast(u32)
        def b16(off, n, t):
            return pltpu.bitcast(wv[t, pl.ds(off // 2, n // 2), :], bf16)
        def ld16(ref, t, r0, n):
            return pltpu.bitcast(ref.bitcast(u32)[t, pl.ds(r0 // 2, n // 2), :], bf16)
        def sp(c, plane): return (c * 6 + plane) * PS
        def ldf(ref, off, n): return jnp.concatenate([ref[t, pl.ds(off, n), :] for t in range(NL)], 1)
        def stf(off, val):
            for t in range(NL):
                sb[t, pl.ds(off, val.shape[0]), :] = val[:, t * 128:(t + 1) * 128]
        vals = {}
        wf[z, pl.ds(0, 8), :] = jnp.zeros((8, 128), f32)
        kvf[z, pl.ds(0, 8), :] = jnp.zeros((8, 128), f32)
        h_v[pl.ds(pl.multiple_of(z * 8, 8), 8), :] = jnp.zeros((8, D), f32)
        hn_v[pl.ds(pl.multiple_of(z * 8, 8), 8), :] = jnp.zeros((8, D), f32)
        x1_v[pl.ds(pl.multiple_of(z * 8, 8), 8), :] = jnp.zeros((8, D), f32)

        def V1(s):
            ins[s][0].wait(); ins[s][1].wait()
            if wmode == 1: ins[s][2].wait(); ins[s][3].wait()
            issue(s + 2)
            shk = shk_ref[...].astype(f32)
            r0 = s * T
            for t in range(NL):
                kf_v[t, pl.ds(8 + r0, T), :] = ld16(k_v, t, r0, T).astype(f32)
            for t in range(NL):
                ks = None
                for j in range(KS):
                    term = kf_v[t, pl.ds(8 + r0 - j, T), :] * shk[j:j + 1, t * 128:(t + 1) * 128]
                    ks = term if ks is None else ks + term
                kvf[t, pl.ds(r0, T), :] = ks * ld16(v_v, t, r0, T).astype(f32)

        def M1(s):
            if wmode == 0: ins[s][2].wait()
            for cc in range(CPS):
                c = s * CPS + cc
                fm = pltpu.bitcast(f_ref.bitcast(u32)[...], bf16)
                u = jnp.dot(fm, ldf(kvf, c * C, C).astype(bf16), preferred_element_type=f32)
                a, b = u[:C], u[C:]
                stf(sp(c, 0), a)
                stf(sp(c, 1), b)
                stf(sp(c, 2), a + b)
                yield 320
                kh = jax.lax.dot_general(fm, pltpu.bitcast(sk_v.bitcast(u32)[c], bf16), (((1,), (1,)), ((), ())),
                                         preferred_element_type=f32)
                cr, dr = kh[:C], kh[C:]
                if c == 0:
                    cf, df = cr, dr
                else:
                    cp, dp = kraw_v[(c - 1) % 2, 0], kraw_v[(c - 1) % 2, 1]
                    Hh = C // 2
                    cf = jnp.concatenate([cr[:Hh] - dp[:Hh], cr[Hh:] + dp[Hh:]], 0)
                    df = jnp.concatenate([dr[:Hh] + cp[:Hh], dr[Hh:] - cp[Hh:]], 0)
                if c + 1 < NC:
                    kraw_v[c % 2, 0] = cr
                    kraw_v[c % 2, 1] = dr
                stf(sp(c, 3), cf)
                stf(sp(c, 4), df - cf)
                stf(sp(c, 5), cf + df)
                yield 320

        def V2(s):
            i0 = s * CPS
            for lb in range(NL):
                for fb in range(C // FR):
                    accs = [None] * CPS
                    kc = {}
                    for j in range(i0 + CPS):
                        uu = [sb[lb, pl.ds(sp(j, x) + fb * FR, FR), :] for x in (2, 0, 1)]
                        for cc in range(CPS):
                            m = i0 + cc - j
                            if m < 0:
                                continue
                            if m not in kc:
                                kc[m] = [sb[lb, pl.ds(sp(m, 3 + x) + fb * FR, FR), :] for x in range(3)]
                            p = [kc[m][x] * uu[x] for x in range(3)]
                            accs[cc] = p if accs[cc] is None else [accs[cc][x] + p[x] for x in range(3)]
                        if j + 1 < i0 + CPS: yield 0
                    outs = []
                    for cc in range(CPS):
                        s1, s2, s3 = accs[cc]
                        wre, wim = s1 - s3, s1 + s2
                        outs += [wre, wim]
                        wf[lb, pl.ds((i0 + cc) * 2 * C + fb * FR, FR), :] = wre
                        wf[lb, pl.ds((i0 + cc) * 2 * C + C + fb * FR, FR), :] = wim
                    sb[z, pl.ds(SROWS - 8, 8), :] = functools.reduce(lambda a, b: a + b, outs)
                    yield 0

        def M2(s):
            if wmode == 0: ins[s][3].wait()
            r0 = s * T
            ys = []
            for cc in range(CPS):
                i = s * CPS + cc
                w = ldf(wf, i * 2 * C, 2 * C).astype(bf16)
                fi = jnp.concatenate([pltpu.bitcast(fi_ref.bitcast(u32)[x], bf16) for x in range(2)], 1)
                ys.append(jnp.dot(fi, w, preferred_element_type=f32))
            y = jnp.concatenate(ys, 0) if CPS > 1 else ys[0]
            sd = sd_ref[...].astype(f32).reshape(1, D)
            y = y + ldf(kvf, r0, T) * sd
            q = jnp.concatenate([ld16(q_v, t, r0, T) for t in range(NL)], 1).astype(f32)
            dq, vq = _center(q)
            h = q + (dq * jax.lax.rsqrt(vq + EPS)) * y
            dh, vh = _center(h)
            r1 = jax.lax.rsqrt(vh + EPS)
            hn = dh * r1
            r2 = jax.lax.rsqrt(vh * r1 * r1 + EPS)
            h_v[pl.ds(r0, T), :] = h
            hn_v[pl.ds(r0, T), :] = hn
            vals["l1", s] = (hn * r2).astype(bf16)
            yield 640

        def M3(s):
            r0 = s * T
            for t in range(NL):
                acc = None
                for kt in range(NL):
                    pr = jnp.dot(vals["l1", s][:, kt * 128:(kt + 1) * 128], b16(H_W1 + kt * 128, 128, t), preferred_element_type=f32)
                    acc = pr if acc is None else acc + pr
                    if kt == NL - 1: g_v[t, pl.ds(8 + r0, T), :] = _gelu(acc)
                    yield T // 4

        def M4(s):
            r0 = s * T
            lane = jax.lax.broadcasted_iota(jnp.int32, (T, 128), 1)
            def ld(t, sh):
                return g_v[t, pl.ds(8 + r0 - sh, T), :]
            tiles = [
                ld(0, 1),
                jnp.where(lane < 32, ld(1, 1), ld(1, -1)),
                jnp.where(lane < 64, ld(2, -1), ld(2, 2)),
                jnp.where(lane < 96, ld(3, 2), ld(3, -2)),
                ld(4, -2),
            ]
            gs = jnp.concatenate(tiles, 1).astype(bf16)
            xs = []
            for t in range(NL):
                acc = hn_v[pl.ds(r0, T), pl.ds(t * 128, 128)]
                for kt in range(NL):
                    acc = acc + jnp.dot(gs[:, kt * 128:(kt + 1) * 128], b16(H_W2 + kt * 128, 128, t), preferred_element_type=f32)
                    yield T // 4
                xs.append(acc)
            x1 = jnp.concatenate(xs, 1)
            d1, v1 = _center(x1)
            vals["ln", s] = (d1 * jax.lax.rsqrt(v1 + EPS)).astype(bf16)
            x1_v[pl.ds(r0, T), :] = x1 + h_v[pl.ds(r0, T), :]

        def M56(s):
            r0 = s * T
            t3s = []
            ln = vals["ln", s]
            if s == 0: wcp[2].wait()
            for t in range(NF):
                acc = None
                for kt in range(NL):
                    pr = jax.lax.dot_general(ln[:, kt * 128:(kt + 1) * 128], b16(H_W3 + t * 128, 128, kt), (((1,), (1,)), ((), ())), preferred_element_type=f32)
                    acc = pr if acc is None else acc + pr
                    if kt == NL - 1: t3s.append(_gelu(acc))
                    yield T // 4
            t3 = jnp.concatenate(t3s, 1).astype(bf16)
            if s == 0: wcp[3].wait()
            for t in range(NL):
                rr = pl.ds(r0, T)
                acc = x1_v[rr, pl.ds(t * 128, 128)]
                for kt in range(NF):
                    acc = acc + jnp.dot(t3[:, kt * 128:(kt + 1) * 128], b16(H_W4 + kt * 128, 128, t), preferred_element_type=f32)
                    if kt == NF - 1: out_v[t, rr, :] = acc.astype(bf16)
                    yield T // 4
            out_copy(s).start()

        def run(g):
            for _ in g: pass

        def chain(*gens):
            for g in gens:
                if g is not None:
                    yield from g

        def interleave(mx, vg, nv):
            pieces_total = mx[1]
            acc = 0.0; done = 0
            for cyc in mx[0]:
                acc += cyc
                want = int(round(min(1.0, acc / pieces_total) * nv))
                while done < want:
                    next(vg); done += 1
            for _ in vg: pass

        def take(g, n):
            if g is None: return
            for _ in range(n):
                yield next(g)

        def waits(s):
            if s < 3:
                for c in ins[s]: c.wait()
            elif s == 3:
                for t in range(3, NS):
                    for c in ins[t]: c.wait()

        NG = (C // FR) * NL
        V1(0); run(M1(0)); run(V2(0))
        for t in range(NS + 2):
            if t < NS: run(M2(t))
            if t + 1 < NS: V1(t + 1)
            m56 = M56(t - 2) if t >= 2 else None
            run(take(m56, lag * NL))
            if t + 1 < NS: run(M1(t + 1))
            if t == 0: wcp[0].wait()
            if t == 1: wcp[1].wait()
            m3 = M3(t) if t < NS else None
            m4 = M4(t - 1) if 1 <= t <= NS else None
            pc = 5 * T // 4
            total = (5 * pc if m4 is not None else 0) + (5 * pc if m3 is not None else 0) + (((NF + NF) * pc - lag * pc) if m56 is not None else 0)
            mx = chain(m3, take(m56, lag2 * NL), m4, m56)
            if t + 1 < NS:
                if total > 0:
                    interleave((mx, total), V2(t + 1), NG * ((t + 2) * CPS))
                else:
                    run(V2(t + 1))
            else:
                run(mx)
        for s in range(NS):
            out_copy(s).wait()

    hb = pl.BlockSpec(memory_space=pltpu.HBM)
    call = pl.pallas_call(
        body,
        out_shape=jax.ShapeDtypeStruct((S, D), bf16),
        in_specs=[hb] * 13,
        out_specs=hb,
        scratch_shapes=[
            pltpu.VMEM((NL, S, 128), bf16), pltpu.VMEM((NL, S, 128), bf16), pltpu.VMEM((NL, S, 128), bf16),
            pltpu.VMEM((NC, D, C), bf16),
            pltpu.VMEM((NL, WROWS, 128), bf16),
            pltpu.VMEM((KS, D), bf16), pltpu.VMEM((D,), bf16), pltpu.VMEM((2 * C, C), bf16), pltpu.VMEM((2, C, C), bf16), pltpu.SMEM((1,), jnp.int32),
            pltpu.VMEM((NL, SROWS, 128), f32),
            pltpu.VMEM((NL, NC * 2 * C, 128), f32),
            pltpu.VMEM((NL, S, 128), f32),
            pltpu.VMEM((NL, S + 8, 128), f32),
            pltpu.VMEM((2, 2, C, D), f32),
            pltpu.VMEM((S, D), f32), pltpu.VMEM((S, D), f32),
            pltpu.VMEM((NL, S + 16, 128), f32),
            pltpu.VMEM((S, D), f32),
            pltpu.VMEM((NL, S, 128), bf16),
            pltpu.SemaphoreType.DMA((NS + 2, 4)), pltpu.SemaphoreType.DMA((NS,)),
        ],
        compiler_params=pltpu.CompilerParams(vmem_limit_bytes=120 * 1024 * 1024),
    )

    def fn(A_q, A_k, A_v, A_shift_k, A_ssm_k, A_ssm_D, B_x, B_w1, B_w2, B_w3, B_w4):
        out = call(A_q.reshape(S, D), A_k.reshape(S, D), A_v.reshape(S, D), A_ssm_k,
                   B_w1, B_w2, B_w3.T, B_w4, A_shift_k.T, A_ssm_D,
                   jnp.asarray(_FWD, bf16), jnp.asarray(_INV, bf16), jnp.zeros((1,), jnp.int32))
        return out.reshape(1, S, D)
    return fn


_fn = build(lag=3, wmode=1)


@jax.jit
def pallas_sequential_preLN__ssm_conv_h3__mixer_s_mlp__prompt_kernel(
    A_q, A_k, A_v, A_shift_k, A_ssm_k, A_ssm_D, B_x, B_w1, B_w2, B_w3, B_w4):
    return _fn(A_q, A_k, A_v, A_shift_k, A_ssm_k, A_ssm_D, B_x, B_w1, B_w2, B_w3, B_w4)
```

```python
import functools
import numpy as np
import jax
import jax.numpy as jnp
import jax.experimental.pallas as pl
import jax.experimental.pallas.tpu as pltpu

S, D, F, KS = 2048, 640, 1728, 4
C = 128
NC = S // C
EPS = 1e-5
NL = D // 128
FP = 1792
NF = FP // 128


def _dft_mats():
    perm = np.concatenate([np.arange(0, C, 2), np.arange(1, C, 2)])
    t = np.arange(C)
    ang = np.outer(2 * perm + 1, t) % (4 * C)
    ang = np.pi * ang / (2 * C)
    fwd = np.concatenate([np.cos(ang), -np.sin(ang)], 0)
    inv = fwd.T / C
    return fwd.astype(np.float32), inv.astype(np.float32)


_FWD, _INV = _dft_mats()
f32, bf16, u32 = jnp.float32, jnp.bfloat16, jnp.uint32


def _gelu(x):
    c0 = float(np.sqrt(2.0 / np.pi))
    c1 = float(np.sqrt(2.0 / np.pi) * 0.044715)
    hx = 0.5 * x
    return hx * jnp.tanh(x * (c0 + c1 * (x * x))) + hx


def _center(x):
    m = jnp.sum(x, axis=-1, keepdims=True) * (1.0 / D)
    d = x - m
    v = jnp.sum(d * d, axis=-1, keepdims=True) * (1.0 / D)
    return d, v

H_W1, H_W2, H_W3, H_W4 = 0, D, 2 * D, 2 * D + FP
WROWS = 2 * D + 2 * FP
PS = C + 8
SROWS = NC * 6 * PS + 8


def build(T=256, lag=3, lag2=2, nodma=0, small=1, wmode=0, order=1, m1pos=2, pk=0, hoist=0, fmin=0, fly=0, kr=0, rh=0, last=99, tiny=0, flat=0, fine0=0, adv=99, only=0):
    NS = S // T
    CPS = T // C
    FR = 8

    def body(q_hbm, k_hbm, v_hbm, sk_hbm, w1_hbm, w2_hbm, w3_hbm, w4_hbm,
             shk_hbm, sd_hbm, f_hbm, fi_hbm, z_hbm,
             out_hbm,
             q_v, k_v, v_v, sk_v, wst, shk_ref, sd_ref, f_ref, fi_ref, z_ref,
             sb, wf, kvf, kf_v, kraw_v, h_v, hn_v, g_v, x1_v, out_v, sems, osems):

        class Multi:
            def __init__(self, cs): self.cs = cs; self.tag = 1
            def start(self):
                if nodma & self.tag: return
                for c in self.cs: c.start()
            def wait(self):
                if nodma & self.tag: return
                for c in self.cs: c.wait()

        def tcopy(src, rows, dst, drows, sem):
            return Multi([pltpu.make_async_copy(src.at[rows, pl.ds(t * 128, 128)], dst.at[t, drows], sem) for t in range(NL)])
        def icopy(src, rows, dst, drows, sem):
            if tiny & 1: rows = drows = pl.ds(rows.start, 16)
            if flat: return Multi([pltpu.make_async_copy(src.at[rows], dst.at[drows], sem)])
            return tcopy(src, rows, dst, drows, sem)
        def in_copies(s):
            rows = pl.ds(s * T, T)
            return [
                icopy(k_hbm, rows, k_v, rows, sems.at[s, 0]),
                icopy(v_hbm, rows, v_v, rows, sems.at[s, 1]),
                Multi([pltpu.make_async_copy(sk_hbm.at[pl.ds(0, 16 if tiny & 1 else D), pl.ds((s * CPS + cc) * C, C)], sk_v.at[s * CPS + cc, pl.ds(0, 16 if tiny & 1 else D)], sems.at[s, 2]) for cc in range(CPS)]),
                icopy(q_hbm, rows, q_v, rows, sems.at[s, 3]),
            ]
        def wcopy(src, off, n, i):
            if tiny & 2: n = 16
            return tcopy(src, pl.ds(0, n), wst, pl.ds(off, n), sems.at[NS, i])
        wcp = [wcopy(w1_hbm, H_W1, D, 0), wcopy(w2_hbm, H_W2, D, 1), wcopy(w3_hbm, H_W3, F, 2), wcopy(w4_hbm, H_W4, F, 3)]
        ccp = Multi([pltpu.make_async_copy(a, b, sems.at[NS + 1, 0]) for a, b in
                     ((shk_hbm, shk_ref), (sd_hbm, sd_ref), (f_hbm, f_ref), (fi_hbm.at[:, pl.ds(0, 128)], fi_ref.at[0]),
                      (fi_hbm.at[:, pl.ds(128, 128)], fi_ref.at[1]), (z_hbm, z_ref))])
        def out_copy(s):
            rows = pl.ds(s * T, T)
            m = Multi([pltpu.make_async_copy(out_v.at[t, rows], out_hbm.at[rows, pl.ds(t * 128, 128)], osems.at[s]) for t in range(NL)])
            m.tag = 4
            return m

        ins = [in_copies(s) for s in range(NS)]
        ccp.tag = 32
        for c in ins[0]: c.tag = 16
        for c in ins[1]: c.tag = 8
        wcp[0].tag = wcp[1].tag = 64
        wcp[2].tag = wcp[3].tag = 2
        ccp.start()
        for c in ins[0]: c.start()
        for c in ins[1][:3]: c.start()
        if order != 3: wcp[0].start()
        if order == 3:
            for c in ins[2][:3]: c.start()
        ins[1][3].start()
        if order == 3: wcp[0].start()
        def issue(s):
            if order == 3 and s < 6: return
            if s < NS:
                for c in ins[s][:3]: c.start()
                ins[s][3].start()
                if 2 <= s <= 4: wcp[s - 1].start()

        g_v[:, pl.ds(0, 8), :] = jnp.zeros((NL, 8, 128), f32)
        g_v[:, pl.ds(S + 8, 8), :] = jnp.zeros((NL, 8, 128), f32)
        kf_v[:, pl.ds(0, 8), :] = jnp.zeros((NL, 8, 128), f32)
        wst[:, pl.ds(H_W3 + F, FP - F), :] = jnp.zeros((NL, FP - F, 128), bf16)
        wst[:, pl.ds(H_W4 + F, FP - F), :] = jnp.zeros((NL, FP - F, 128), bf16)
        ccp.wait()
        z = z_ref[0]

        wv = wst.bitcast(u32)
        def b16(off, n, t):
            return pltpu.bitcast(wv[t, pl.ds(off // 2, n // 2), :], bf16)
        def ld16(ref, t, r0, n):
            if flat: return ref[pl.ds(r0, n), pl.ds(t * 128, 128)]
            return pltpu.bitcast(ref.bitcast(u32)[t, pl.ds(r0 // 2, n // 2), :], bf16)
        def sp(c, plane): return (c * 6 + plane) * PS
        def ldf(ref, off, n): return jnp.concatenate([ref[t, pl.ds(off, n), :] for t in range(NL)], 1)
        def stf(off, val):
            for t in range(NL):
                sb[t, pl.ds(off, val.shape[0]), :] = val[:, t * 128:(t + 1) * 128]
        vals = {}
        wf[z, pl.ds(0, 8), :] = jnp.zeros((8, 128), f32)
        kvf[z, pl.ds(0, 8), :] = jnp.zeros((8, 128), f32)
        h_v[pl.ds(pl.multiple_of(z * 8, 8), 8), :] = jnp.zeros((8, D), f32)
        hn_v[pl.ds(pl.multiple_of(z * 8, 8), 8), :] = jnp.zeros((8, D), f32)
        x1_v[pl.ds(pl.multiple_of(z * 8, 8), 8), :] = jnp.zeros((8, D), f32)

        hook = {}
        synced = set()
        def sync(s):
            if s < NS and s not in synced:
                synced.add(s)
                if s + 1 == last:
                    for s2 in range(s + 2, NS): issue(s2)
                elif s < last: issue(s + 2)
                for c in (ins[s] if s >= fine0 else ins[s][:2]): c.wait()
                if s >= last:
                    for s2 in range(s + 1, NS):
                        synced.add(s2)
                        for c in ins[s2]: c.wait()

        def V1(s):
            if order == 1 and (wmode == 1 or s == 0 or (wmode in (5, 6) and s == 1)):
                sync(s)
            shk = shk_ref[...].astype(f32)
            r0 = s * T
            for t in range(NL):
                kf_v[t, pl.ds(8 + r0, T), :] = ld16(k_v, t, r0, T).astype(f32)
            for t in range(NL):
                ks = None
                for j in range(KS):
                    term = kf_v[t, pl.ds(8 + r0 - j, T), :] * shk[j:j + 1, t * 128:(t + 1) * 128]
                    ks = term if ks is None else ks + term
                kvf[t, pl.ds(r0, T), :] = ks * ld16(v_v, t, r0, T).astype(f32)

        def M1(s):
            if s < (4 if order == 3 else fine0): ins[s][2].wait()
            for cc in range(CPS):
                c = s * CPS + cc
                fm = pltpu.bitcast(f_ref.bitcast(u32)[...], bf16)
                u = jnp.dot(fm, ldf(kvf, c * C, C).astype(bf16), preferred_element_type=f32)
                a, b = u[:C], u[C:]
                stf(sp(c, 0), a)
                stf(sp(c, 1), b)
                if not fly: stf(sp(c, 2), a + b)
                yield 320
                kh = jax.lax.dot_general(fm, pltpu.bitcast(sk_v.bitcast(u32)[c], bf16), (((1,), (1,)), ((), ())),
                                         preferred_element_type=f32)
                cr, dr = kh[:C], kh[C:]
                if c == 0:
                    cf, df = cr, dr
                else:
                    cp, dp = (kraw_v[0, 0], kraw_v[0, 1]) if (cc == 0 or not kr) else prev
                    Hh = C // 2
                    cf = jnp.concatenate([cr[:Hh] - dp[:Hh], cr[Hh:] + dp[Hh:]], 0)
                    df = jnp.concatenate([dr[:Hh] + cp[:Hh], dr[Hh:] - cp[Hh:]], 0)
                prev = (cr, dr)
                if c + 1 < NC and (cc == CPS - 1 or not kr):
                    kraw_v[0, 0] = cr
                    kraw_v[0, 1] = dr
                stf(sp(c, 3), cf)
                stf(sp(c, 4), df - cf)
                stf(sp(c, 5), cf + df)
                yield 320

        def V2(s):
            i0 = s * CPS
            for lb in range(NL):
                for fb in range(C // FR):
                    accs = [None] * CPS
                    kc = {}
                    for j in range(i0 + CPS):
                        if fly:
                            uu = [sb[lb, pl.ds(sp(j, x) + fb * FR, FR), :] for x in (0, 1)]
                            uu = [uu[0] + uu[1]] + uu
                        else:
                            uu = [sb[lb, pl.ds(sp(j, x) + fb * FR, FR), :] for x in (2, 0, 1)]
                        for cc in range(CPS):
                            m = i0 + cc - j
                            if m < 0:
                                continue
                            if m not in kc:
                                kc[m] = [sb[lb, pl.ds(sp(m, 3 + x) + fb * FR, FR), :] for x in range(3)]
                            p = [kc[m][x] * uu[x] for x in range(3)]
                            accs[cc] = p if accs[cc] is None else [accs[cc][x] + p[x] for x in range(3)]
                        if j + 1 < i0 + CPS: yield 0
                    outs = []
                    for cc in range(CPS):
                        s1, s2, s3 = accs[cc]
                        wre, wim = s1 - s3, s1 + s2
                        outs += [wre, wim]
                        wf[lb, pl.ds((i0 + cc) * 2 * C + fb * FR, FR), :] = wre
                        wf[lb, pl.ds((i0 + cc) * 2 * C + C + fb * FR, FR), :] = wim
                    if s >= fmin: sb[z, pl.ds(SROWS - 8, 8), :] = functools.reduce(lambda a, b: a + b, outs)
                    yield 0

        def M2(s):
            if wmode == 2: sync(s + 1)
            if s < (3 if order == 3 else fine0): ins[s][3].wait()
            r0 = s * T
            ys = []
            for cc in range(CPS):
                i = s * CPS + cc
                w = ldf(wf, i * 2 * C, 2 * C).astype(bf16)
                fi = jnp.concatenate([pltpu.bitcast(fi_ref.bitcast(u32)[x], bf16) for x in range(2)], 1)
                ys.append(jnp.dot(fi, w, preferred_element_type=f32))
            y = jnp.concatenate(ys, 0) if CPS > 1 else ys[0]
            if wmode == 3: sync(s + 1); sync(s + 2 if s >= adv else 0)
            sd = sd_ref[...].astype(f32).reshape(1, D)
            y = y + ldf(kvf, r0, T) * sd
            q = jnp.concatenate([ld16(q_v, t, r0, T) for t in range(NL)], 1).astype(f32)
            dq, vq = _center(q)
            h = q + (dq * jax.lax.rsqrt(vq + EPS)) * y
            if wmode == 4: sync(s + 1); sync(s + 2 if s >= adv else 0)
            if s in hook: hook[s]()
            mh = jnp.sum(h, axis=-1, keepdims=True) * (1.0 / D)
            dh = h - mh
            vh = jnp.sum(dh * dh, axis=-1, keepdims=True) * (1.0 / D)
            r1 = jax.lax.rsqrt(vh + EPS)
            hn = dh * r1
            r2 = jax.lax.rsqrt(vh * r1 * r1 + EPS)
            h_v[pl.ds(r0, T), :] = h
            if rh: vals["st", s] = (mh, r1)
            else: hn_v[pl.ds(r0, T), :] = hn
            vals["l1", s] = (hn * r2).astype(bf16)
            yield 640

        def M3(s):
            r0 = s * T
            for t in range(NL):
                acc = None
                for kt in range(NL):
                    pr = jnp.dot(vals["l1", s][:, kt * 128:(kt + 1) * 128], b16(H_W1 + kt * 128, 128, t), preferred_element_type=f32)
                    acc = pr if acc is None else acc + pr
                    if kt == NL - 1: g_v[t, pl.ds(8 + r0, T), :] = _gelu(acc)
                    yield T // 4

        def M4(s):
            r0 = s * T
            lane = jax.lax.broadcasted_iota(jnp.int32, (T, 128), 1)
            def ld(t, sh):
                return g_v[t, pl.ds(8 + r0 - sh, T), :]
            tiles = [
                ld(0, 1),
                jnp.where(lane < 32, ld(1, 1), ld(1, -1)),
                jnp.where(lane < 64, ld(2, -1), ld(2, 2)),
                jnp.where(lane < 96, ld(3, 2), ld(3, -2)),
                ld(4, -2),
            ]
            gs = jnp.concatenate(tiles, 1).astype(bf16)
            xs = []
            for t in range(NL):
                if rh: acc = (h_v[pl.ds(r0, T), pl.ds(t * 128, 128)] - vals["st", s][0]) * vals["st", s][1]
                else: acc = hn_v[pl.ds(r0, T), pl.ds(t * 128, 128)]
                for kt in range(NL):
                    acc = acc + jnp.dot(gs[:, kt * 128:(kt + 1) * 128], b16(H_W2 + kt * 128, 128, t), preferred_element_type=f32)
                    yield T // 4
                xs.append(acc)
            x1 = jnp.concatenate(xs, 1)
            d1, v1 = _center(x1)
            vals["ln", s] = (d1 * jax.lax.rsqrt(v1 + EPS)).astype(bf16)
            x1_v[pl.ds(r0, T), :] = x1 + h_v[pl.ds(r0, T), :]

        def M56(s):
            r0 = s * T
            t3s = []
            ln = vals["ln", s]
            if s == 0: wcp[2].wait()
            for t in range(NF):
                acc = None
                for kt in range(NL):
                    pr = jax.lax.dot_general(ln[:, kt * 128:(kt + 1) * 128], b16(H_W3 + t * 128, 128, kt), (((1,), (1,)), ((), ())), preferred_element_type=f32)
                    acc = pr if acc is None else acc + pr
                    if kt == NL - 1: t3s.append(_gelu(acc).astype(bf16) if pk else _gelu(acc))
                    yield T // 4
            t3 = None if pk else jnp.concatenate(t3s, 1).astype(bf16)
            if s == 0: wcp[3].wait()
            for t in range(NL):
                if wmode >= 10 and t == wmode - 10: sync(s + 4)
                rr = pl.ds(r0, T)
                acc = x1_v[rr, pl.ds(t * 128, 128)]
                for kt in range(NF):
                    acc = acc + jnp.dot(t3s[kt] if pk else t3[:, kt * 128:(kt + 1) * 128], b16(H_W4 + kt * 128, 128, t), preferred_element_type=f32)
                    if kt == NF - 1: out_v[t, rr, :] = acc.astype(bf16)
                    yield T // 4
            out_copy(s).start()

        def run(g):
            for _ in g: pass

        def chain(*gens):
            for g in gens:
                if g is not None:
                    yield from g

        def interleave(mx, vg, nv):
            pieces_total = mx[1]
            acc = 0.0; done = 0
            for cyc in mx[0]:
                acc += cyc
                want = int(round(min(1.0, acc / pieces_total) * nv))
                while done < want:
                    next(vg); done += 1
            for _ in vg: pass

        def take(g, n):
            if g is None: return
            for _ in range(n):
                yield next(g)

        def waits(s):
            if s < 3:
                for c in ins[s]: c.wait()
            elif s == 3:
                for t in range(3, NS):
                    for c in ins[t]: c.wait()

        NG = (C // FR) * NL
        def steady(t, skip=()):
            if t < NS and "M2" not in skip: run(M2(t))
            if t + 1 < NS and "M1" not in skip: V1(t + 1)
            m56 = M56(t - 2) if t >= 2 else None
            m3 = M3(t) if t < NS else None
            if "M1" in skip:
                first, m3 = m3, None
                run(first)
            run(take(m56, lag * NL))
            if t + 1 < NS and "M1" not in skip: run(M1(t + 1))
            m4 = M4(t - 1) if 1 <= t <= NS else None
            pc = 5 * T // 4
            total = (5 * pc if m4 is not None else 0) + (5 * pc if m3 is not None else 0) + (((NF + NF) * pc - lag * pc) if m56 is not None else 0)
            mx = chain(m3, take(m56, lag2 * NL), m4, m56)
            if t + 1 < NS:
                interleave((mx, total), V2(t + 1), NG * ((t + 2) * CPS))
            else:
                run(mx)
        if order == 3:
            def W(*cs):
                for c in cs: c.wait()
            synced.update([0, 1, 2, 3])
            W(ins[0][0], ins[0][1]); V1(0); run(M1(0))
            for c in ins[3][:3]: c.start()
            ins[2][3].start(); wcp[1].start()
            W(*ins[1][:2]); run(V2(0)); V1(1); run(M1(1))
            wcp[2].start(); ins[3][3].start()
            if hoist & 2: W(*ins[2][:2]); V1(2)
            else: hook[0] = lambda: W(*ins[2][:2])
            run(M2(0))
            if not hoist & 2: V1(2)
            run(M1(2)); run(V2(1))
            for c in ins[4]: c.start()
            hook[1] = lambda: W(wcp[0], *(ins[3][:2] if hoist & 1 else []))
            run(M2(1))
            if hoist & 1: V1(3)
            interleave((chain(M3(0), M3(1)), 2 * 5 * 5 * T // 4), V2(2), NG * 3 * CPS)
            wcp[3].start()
            if not hoist & 1: W(*ins[3][:2]); V1(3)
            run(M1(3))
            for c in ins[5]: c.start()
            hook[2] = lambda: W(wcp[1], ins[3][3])
            run(M2(2)); run(M4(0))
            steady(2, ("M2", "M1"))
            for t in range(3, NS + 2): steady(t)
        elif order == 1:
            V1(0); run(M1(0)); run(V2(0))
            for t in range(NS + 2):
                if wmode >= 10: sync(t + 1)
                if t < NS: run(M2(t))
                if t + 1 < NS and t <= adv: V1(t + 1)
                if t + 2 < NS and t >= adv: V1(t + 2)
                m56 = M56(t - 2) if t >= 2 else None
                run(take(m56, lag * NL))
                if wmode == 5: sync(t + 2)
                if t + 1 < NS: run(M1(t + 1))
                if wmode == 6: sync(t + 2)
                if t == 0: wcp[0].wait()
                if t == 1: wcp[1].wait()
                m3 = M3(t) if t < NS else None
                m4 = M4(t - 1) if 1 <= t <= NS else None
                pc = 5 * T // 4
                total = (5 * pc if m4 is not None else 0) + (5 * pc if m3 is not None else 0) + (((NF + NF) * pc - lag * pc) if m56 is not None else 0)
                mx = chain(m3, take(m56, lag2 * NL), m4, m56)
                if t + 1 < NS:
                    if total > 0:
                        interleave((mx, total), V2(t + 1), NG * ((t + 2) * CPS))
                    else:
                        run(V2(t + 1))
                else:
                    run(mx)

        else:
            def V1M1(s):
                if s < NS:
                    sync(s); V1(s)
                    yield from M1(s)
            run(V1M1(0)); run(V2(0)); run(V1M1(1))
            for t in range(NS + 2):
                if t < NS: run(M2(t))
                m56 = M56(t - 2) if t >= 2 else None
                if t == 0: wcp[0].wait()
                if t == 1: wcp[1].wait()
                m3 = M3(t) if t < NS else None
                m4 = M4(t - 1) if 1 <= t <= NS else None
                pc = 5 * T // 4
                total = (5 * pc if m4 is not None else 0) + (5 * pc if m3 is not None else 0) + ((NF * pc + m1pos * NF * T // 4) if m56 is not None else 0)
                mx = chain(take(m56, lag * NL), m3, take(m56, lag2 * NL), m4, take(m56, (NF - lag - lag2) * NL + m1pos * NF))
                if t + 1 < NS and total > 0:
                    interleave((mx, total), V2(t + 1), NG * ((t + 2) * CPS))
                else:
                    run(mx)
                run(V1M1(t + 2))
                run(m56 or [])
        for s in range(NS):
            out_copy(s).wait()

    hb = pl.BlockSpec(memory_space=pltpu.HBM)
    call = pl.pallas_call(
        body,
        out_shape=jax.ShapeDtypeStruct((S, D), bf16),
        in_specs=[hb] * 13,
        out_specs=hb,
        scratch_shapes=[
            *[pltpu.VMEM((S, D) if flat else (NL, S, 128), bf16) for _ in range(3)],
            pltpu.VMEM((NC, D, C), bf16),
            pltpu.VMEM((NL, WROWS, 128), bf16),
            pltpu.VMEM((KS, D), bf16), pltpu.VMEM((D,), bf16), pltpu.VMEM((2 * C, C), bf16), pltpu.VMEM((2, C, C), bf16), pltpu.SMEM((1,), jnp.int32),
            pltpu.VMEM((NL, SROWS, 128), f32),
            pltpu.VMEM((NL, NC * 2 * C, 128), f32),
            pltpu.VMEM((NL, S, 128), f32),
            pltpu.VMEM((NL, S + 8, 128), f32),
            pltpu.VMEM((2, 2, C, D), f32),
            pltpu.VMEM((S, D), f32), pltpu.VMEM((S, D), f32),
            pltpu.VMEM((NL, S + 16, 128), f32),
            pltpu.VMEM((S, D), f32),
            pltpu.VMEM((NL, S, 128), bf16),
            pltpu.SemaphoreType.DMA((NS + 2, 4)), pltpu.SemaphoreType.DMA((NS,)),
        ],
        compiler_params=pltpu.CompilerParams(vmem_limit_bytes=120 * 1024 * 1024),
    )

    def fn(A_q, A_k, A_v, A_shift_k, A_ssm_k, A_ssm_D, B_x, B_w1, B_w2, B_w3, B_w4):
        out = call(A_q.reshape(S, D), A_k.reshape(S, D), A_v.reshape(S, D), A_ssm_k,
                   B_w1, B_w2, B_w3.T, B_w4, A_shift_k.T, A_ssm_D,
                   jnp.asarray(_FWD, bf16), jnp.asarray(_INV, bf16), jnp.zeros((1,), jnp.int32))
        return out.reshape(1, S, D)
    return fn


_fn = build(lag=4, wmode=4, fine0=2, flat=1, last=6, fmin=1, pk=1, order=1, fly=1)


@jax.jit
def pallas_sequential_preLN__ssm_conv_h3__mixer_s_mlp__prompt_kernel(
    A_q, A_k, A_v, A_shift_k, A_ssm_k, A_ssm_D, B_x, B_w1, B_w2, B_w3, B_w4):
    return _fn(A_q, A_k, A_v, A_shift_k, A_ssm_k, A_ssm_D, B_x, B_w1, B_w2, B_w3, B_w4)
```
